```python
import jax
import jax.numpy as jnp

def _softmax(x, axis=-1):
    return jax.nn.softmax(x, axis=axis)

def _gelu(x):
    return jax.nn.gelu(x, approximate=True)

def _silu(x):
    return jax.nn.silu(x)

def _sigmoid(x):
    return jax.nn.sigmoid(x)

def _layernorm(x, axis=-1, eps=1e-05):
    m = jnp.mean(x, axis=axis, keepdims=True)
    v = jnp.var(x, axis=axis, keepdims=True)
    return (x - m) / jnp.sqrt(v + eps)

def _scatter_add(tgt, idx, src, axis=0):
    return tgt.at[idx].add(src)

def _segment_sum(src, seg, n):
    return jax.ops.segment_sum(src, seg, n)

class _Rng:

    def __init__(self, key):
        self._k = key

    def _next(self):
        self._k, sub = jax.random.split(self._k)
        return sub

    def normal(self, shape):
        return jax.random.normal(self._next(), shape, dtype=jnp.bfloat16)

    def randint(self, lo, hi, shape):
        return jax.random.randint(self._next(), shape, lo, hi, dtype=jnp.int32)

    def uniform(self, shape, lo=0.0, hi=1.0):
        return jax.random.uniform(self._next(), shape, jnp.bfloat16, lo, hi)

    def permutation(self, n):
        return jax.random.permutation(self._next(), n)
kernel_name = 'adaLN_cond__grouped_kv_mqa__mixer_token_mlp__prompt'

def _fwd_setup_inputs():
    _rng = _Rng(jax.random.key(int.from_bytes(__import__("os").urandom(4), "little")))
    _w = lambda a: (lambda t: t.astype(jnp.bfloat16) if jnp.issubdtype(t.dtype, jnp.floating) else t)(jnp.asarray(a))

    def _A_setup():
        B, S, D, H = (1, 2048, 512, 32)
        Dh = D // H
        return {'x': _w((lambda *s: _rng.normal(s) * 0.05)(B, S, D)), 'wq': _w((lambda *s: _rng.normal(s) * 0.05)(D, H * Dh)), 'wk': _w((lambda *s: _rng.normal(s) * 0.05)(D, Dh)), 'wv': _w((lambda *s: _rng.normal(s) * 0.05)(D, Dh)), 'wo': _w((lambda *s: _rng.normal(s) * 0.05)(H * Dh, D))}
    _A_in = _A_setup()

    def _B_setup():
        B, S, D, F = (1, 2048, 512, 1376)
        return {'x': _w((lambda *s: _rng.normal(s) * 0.05)(B, S, D)), 'w1': _w((lambda *s: _rng.normal(s) * 0.05)(S, F) * S ** (-0.5)), 'b1': _w((lambda *s: _rng.normal(s) * 0.05)(F) * 0.02), 'w2': _w((lambda *s: _rng.normal(s) * 0.05)(F, S) * F ** (-0.5)), 'b2': _w((lambda *s: _rng.normal(s) * 0.05)(S) * 0.02)}
    _B_in = _B_setup()
    return {'A_x': _A_in['x'], 'A_wq': _A_in['wq'], 'A_wk': _A_in['wk'], 'A_wv': _A_in['wv'], 'A_wo': _A_in['wo'], 'B_x': _B_in['x'], 'B_w1': _B_in['w1'], 'B_b1': _B_in['b1'], 'B_w2': _B_in['w2'], 'B_b2': _B_in['b2'], 'c': _w((lambda *s: _rng.normal(s) * 0.05)(1, 512)), 'w_mod': _w((lambda *s: _rng.normal(s) * 0.05)(512, 6 * 512) * 512 ** (-0.5))}

def _fwd_reference(A_x, A_wq, A_wk, A_wv, A_wo, B_x, B_w1, B_b1, B_w2, B_b2, c, w_mod):

    def _A_ref(x, wq, wk, wv, wo):
        B, S, D = x.shape
        H = 32
        Dh = D // H
        q = (lambda x, *d: x.transpose(*d))((x @ wq).reshape(B, S, H, Dh), 0, 2, 1, 3)
        k = x @ wk
        v = x @ wv
        scores = jnp.einsum('bhqd,bkd->bhqk', q, k) * Dh ** (-0.5)
        p = _softmax(scores, axis=-1)
        o = jnp.einsum('bhqk,bkd->bhqd', p, v)
        return (lambda x, *d: x.transpose(*d))(o, 0, 2, 1, 3).reshape(B, S, H * Dh) @ wo

    def _B_ref(x, w1, b1, w2, b2):
        B, S, D = x.shape
        h = _layernorm(x, axis=-1)
        u = jnp.einsum('bsd,sf->bdf', h, w1) + b1
        u = _gelu(u)
        y = jnp.einsum('bdf,fs->bds', u, w2) + b2
        return (lambda x, *d: x.transpose(*d))(y, 0, 2, 1)
    x = A_x
    mod = (_silu(c) @ w_mod).reshape(c.shape[0], 6, 1, -1)
    sa, ca, ga, sb, cb, gb = (mod[:, 0].copy(), mod[:, 1].copy(), mod[:, 2].copy(), mod[:, 3].copy(), mod[:, 4].copy(), mod[:, 5].copy())
    h = _layernorm(x, axis=-1) * (1 + ca) + sa
    x = x + ga * _A_ref(h, A_wq, A_wk, A_wv, A_wo)
    h = _layernorm(x, axis=-1) * (1 + cb) + sb
    x = x + gb * _B_ref(h, B_w1, B_b1, B_w2, B_b2)
    return x

def setup_inputs():
    _inp = _fwd_setup_inputs()
    _gk = jax.random.fold_in(jax.random.key(int.from_bytes(__import__("os").urandom(4), "little")), 2 ** 31 - 1)
    _shapes = [[1, 2048, 512]]
    _dtypes = ['bfloat16']
    _gks = jax.random.split(_gk, len(_shapes))
    _gs = [jax.random.normal(k, s, dtype=jnp.dtype(d)) * 0.05 for k, s, d in zip(_gks, _shapes, _dtypes)]
    _inp['grad_out'] = _gs[0]
    return _inp

def reference(A_x, A_wq, A_wk, A_wv, A_wo, B_w1, B_b1, B_w2, B_b2, c, w_mod, B_x, grad_out):
    _const = dict(B_x=B_x)

    def _f(*_d):
        return _fwd_reference(**{'A_x': _d[0], 'A_wq': _d[1], 'A_wk': _d[2], 'A_wv': _d[3], 'A_wo': _d[4], 'B_w1': _d[5], 'B_b1': _d[6], 'B_w2': _d[7], 'B_b2': _d[8], 'c': _d[9], 'w_mod': _d[10], **_const})
    _out, _vjp = jax.vjp(_f, A_x, A_wq, A_wk, A_wv, A_wo, B_w1, B_b1, B_w2, B_b2, c, w_mod)
    _grads = _vjp(grad_out)
    _out0 = jnp.asarray(_out)
    return (_out0, *[jnp.asarray(_g) for _g in _grads])
```

```python
import math

import jax
import jax.numpy as jnp
import jax.experimental.pallas as pl
import jax.experimental.pallas.tpu as pltpu

F32 = jnp.float32
BF16 = jnp.bfloat16
U32 = jnp.uint32

S = 2048
D = 512
H = 32
DH = 16
F = 1376
FP = 1408
ROWS = (176, 176, 176, 160)
QB = 512
NB = S // QB
NT128 = QB // 128
NU = NB * H
BK = 128
NJ = S // BK
U = 4
GB = H // U
NG = NU // U
PAIR = 2
UB = PAIR * U
LAG = 3
NSLOT = 13
NREC = 3
REC0 = GB - NREC
NSPILL = NG - NREC - NSLOT
EXTRA = 1536
PACE = 24

EPS = 1e-5
LOG2E = math.log2(math.e)
SM_SCALE = DH ** -0.5
SAFE_BOUND = 40.0
GELU_C = math.sqrt(2.0 / math.pi)
GELU_A = 0.044715

NN = (((1,), (0,)), ((), ()))
NT = (((1,), (1,)), ((), ()))


def _dot(a, b, dims=NN):
    return jax.lax.dot_general(a, b, dims, preferred_element_type=F32)


def _plus(x, y, sign=1):
    x, y = x.astype(F32), y.astype(F32)
    return (x + y if sign > 0 else x - y).astype(BF16)


def _strassen_rhs(b):
    k, n = b.shape[0] // 2, b.shape[1] // 2
    b11, b12, b21, b22 = b[0:k, 0:n], b[0:k, n:], b[k:, 0:n], b[k:, n:]
    return (_plus(b11, b22), b11, _plus(b12, b22, -1), _plus(b21, b11, -1), b22,
            _plus(b11, b12), _plus(b21, b22))


def _strassen(top, bottom, rhs):
    k = top.shape[1] // 2
    a11, a12, a21, a22 = top[:, 0:k], top[:, k:], bottom[:, 0:k], bottom[:, k:]
    lhs = (_plus(a11, a22), _plus(a21, a22), a11, a22, _plus(a11, a12),
           _plus(a21, a11, -1), _plus(a12, a22, -1))
    p1, p2, p3, p4, p5, p6, p7 = (_dot(l, r) for l, r in zip(lhs, rhs))
    return (jnp.concatenate([p1 + p4 - p5 + p7, p3 + p5], axis=1),
            jnp.concatenate([p2 + p4, p1 - p2 + p3 + p6], axis=1))


def _col(row):
    return jnp.broadcast_to(row, (128, row.shape[1])).T


def _row(acc):
    return jnp.sum(acc.T, axis=0, keepdims=True)


def _wide(col):
    return jnp.tile(col, (1, NT128))


def _sum0(x):
    return jnp.broadcast_to(jnp.sum(x, axis=0, keepdims=True), x.shape)


def _layernorm(x):
    mu = jnp.sum(x, axis=0, keepdims=True) * (1.0 / D)
    xc = x - mu
    r = jax.lax.rsqrt(jnp.sum(xc * xc, axis=0, keepdims=True) * (1.0 / D) + EPS)
    return mu, r, xc * r


def _aligned(i, n):
    return i if isinstance(i, int) else pl.multiple_of(i, n)


def _span(i, n):
    return pl.ds(_aligned(i * n, n), n)


def _lanes(t):
    return slice(t * 128, (t + 1) * 128)


def _start(copies, **kwargs):
    for cp in copies:
        cp.start(**kwargs)


def _wait(copies):
    for cp in copies:
        cp.wait()


def _true(i):
    return jnp.full((8, 128), i) < NU


def _after(words, deps, always):
    nr, nc = words.shape[0] // 8, words.shape[1] // 128
    cols = []
    for c in range(nc):
        tiles = []
        for r in range(nr):
            tile = words[r * 8:(r + 1) * 8, _lanes(c)]
            n = c * nr + r
            for dep in deps[n * len(deps) // (nr * nc):(n + 1) * len(deps) // (nr * nc)][-1:]:
                tile = jnp.where(always, tile, pltpu.bitcast(dep, U32))
            tiles.append(tile)
        cols.append(jnp.concatenate(tiles, axis=0))
    return jnp.concatenate(cols, axis=1)


def _tie(words, deps, always):
    if deps:
        head = jnp.where(always, words[:, 0:128], pltpu.bitcast(deps.pop(0), U32))
        words = head if words.shape[1] == 128 else jnp.concatenate([head, words[:, 128:]], axis=1)
    return pltpu.bitcast(words, BF16)


def _vpu_scores(cols_ref, rows_ref, init, shares, width):
    cols = cols_ref[...]
    sums = [init]
    for i in range(DH):
        row = jnp.concatenate([jnp.broadcast_to(rows_ref[i:i + 1, _lanes(t)], (16, 128))
                               for t in range(NT128)], axis=1)
        sums.append(sums[-1] + jnp.concatenate([cols[i]] * NT128, axis=1) * row)
    chain = [(a, t) for t in range(width - 1, NT128, width) for a in sums[1:]]
    picks = [chain[max(round(sum(shares[:n + 1]) * len(chain) / sum(shares)) - 1, 0)]
             for n in range(len(shares))]
    return sums[-1], [a[8:16, _lanes(t)] for a, t in picks]


def _kept(g):
    return jnp.where(g < REC0, g, jnp.maximum(g - NREC, REC0))


def _slot(i):
    return i - NSLOT * sum((i >= n).astype(jnp.int32) for n in range(NSLOT, NG, NSLOT))


def _spills_before(g):
    return jnp.minimum(jnp.minimum((g * NSPILL + PACE - 1) // PACE, _kept(g)), NSPILL)


assert NSPILL <= PACE < NG and all(
    min(-(-g * NSPILL // PACE), g - NREC, NSPILL) > g - NREC - NSLOT for g in range(GB, NG))
assert NREC <= GB // 2 and GB + 3 < NSLOT and GB + 2 + NREC <= NSLOT


def _kernel(x_hbm, wq_hbm, wkt_hbm, wvt_hbm, wo_hbm, w1_hbm, b1_hbm, w2_hbm, b2_hbm,
            c_hbm, wmod_hbm, go_hbm,
            out_hbm, dx_hbm, dwq_hbm, dwkt_hbm, dwvt_hbm, dwo_hbm, dw1_hbm, db1_hbm,
            dw2_hbm, db2_hbm, dc_hbm, dwmod_hbm, p_hbm,
            ring, p_extra, x1t, qt, ot, kt_s, vt_s, rowv, shift, stat, mod_s, dmod_s, colv,
            w1b, dut, gt, gob, gacc, acc_s,
            wkt_ref, wvt_ref, b1_ref, b2_ref, c_ref, bounded, p_sem, sem):

    def mod_row(i):
        return mod_s[i]

    def heads(ref, b):
        return ref[pl.ds(b * H, H)].reshape(D, QB)

    def keys(ref, j):
        return ref[j // NT128, :, _lanes(j % NT128)]

    def key_buffers():
        return pltpu.VMEM((S // 2, 128), U32), pltpu.VMEM((NJ, DH, 16, 128), F32)

    def build_keys(src, rows, cols):
        last = []
        for b in range(NB):
            k = pltpu.bitcast(
                jnp.concatenate([src[b], jnp.ones((128 - DH, QB), BF16)], axis=0).T, U32)
            rows[b * QB // 2:(b + 1) * QB // 2, :] = k
            last += [k[(t + 1) * BK // 2 - 8:(t + 1) * BK // 2] for t in range(NT128)]
        last = pltpu.bitcast(jnp.concatenate(last, axis=0), BF16)[:, 0:DH]
        for i0 in range(0, DH, 4):
            pick = (jax.lax.broadcasted_iota(jnp.int32, (DH, 4 * 128), 0)
                    == i0 + jax.lax.broadcasted_iota(jnp.int32, (DH, 4 * 128), 1) // 128)
            out = _dot(last, jnp.where(pick, 1.0, 0.0).astype(BF16))
            for i in range(4):
                cols[:, i0 + i] = out[:, _lanes(i)].reshape(NJ, 16, 128)

    def key_rows(src, j, lo, hi, width, deps, always):
        return jnp.concatenate(
            [_tie(src[(j * BK + r) // 2:(j * BK + r) // 2 + 8, :], deps, always)
             for r in range(lo, hi, 16)], axis=0)[:, 0:width]

    def scores(src, u, j):
        return _dot(pltpu.bitcast(src[_span(j, BK // 2), :], BF16)[:, 0:DH], qt[u])

    def spare(slot, row, n):
        return ring.at[slot, row:row + n, :]

    xb = spare(GB, 0, S)
    wm_all = spare(GB, S, 6 * D)
    wqb = spare(GB, S + 6 * D, D)
    wob = spare(GB, S + 7 * D, D)
    go_all = spare(GB + 2, S, S)
    w2_all = [spare(GB + 3, b * S, F) for b in range(NB)]
    dwm_all = spare(GB + 1, 0, 6 * D)
    dwqb = spare(GB + 1, 7 * D, D)
    wot = gt.at[0:D, :]
    wqt = gt.at[D:2 * D, :]
    dwob = w1b.at[0:D, :]

    def p_move(cond, i, spill, act):
        for first in (True, False):
            @pl.when(jnp.logical_and(cond, (i == 0) == first))
            def _():
                n = U * S - first * EXTRA
                base = (NSPILL - 1) * U * S if first else pl.multiple_of((i - 1) * U * S, S)
                ends = ring.at[_slot(i), 0:n, :], p_hbm.at[pl.ds(base, n), :]
                act(pltpu.make_async_copy(*(ends if spill else ends[::-1]), p_sem.at[_slot(i)]))
                if first:
                    ends = ring.at[0, n:U * S, :], p_extra
                    act(pltpu.make_async_copy(*(ends if spill else ends[::-1]), p_sem.at[NSLOT]))

    def x_copy(b):
        return pltpu.make_async_copy(
            x_hbm.at[0, _span(b, QB), :], xb.at[_span(b, QB), :], sem.at[1 + b])

    def wmod_copy(i):
        return pltpu.make_async_copy(
            wmod_hbm.at[:, _span(i, D)], wm_all.at[_span(i, D), :], sem.at[5 + i])

    def wq_copy():
        return pltpu.make_async_copy(wq_hbm, wqb, sem.at[11])

    def go_copy(b):
        return pltpu.make_async_copy(go_hbm.at[0, _span(b, QB), :], gob, sem.at[13])

    small = ((c_hbm, c_ref, dc_hbm), (b1_hbm, b1_ref, db1_hbm), (wkt_hbm, wkt_ref, dwkt_hbm),
             (wvt_hbm, wvt_ref, dwvt_hbm), (b2_hbm, b2_ref, db2_hbm))
    small_in = [pltpu.make_async_copy(src, ref, sem.at[23 + n])
                for n, (src, ref, _) in enumerate(small)]
    small_out = [pltpu.make_async_copy(ref, dst, sem.at[23 + n])
                 for n, (_, ref, dst) in enumerate(small)]
    _start(small_in + [wmod_copy(0), wmod_copy(1), x_copy(0), x_copy(1)])
    _wait(small_in)
    c32 = c_ref[...].astype(F32)
    sig = jax.nn.sigmoid(c32)
    silu_c = c32 * sig

    def modulation(w):
        return _dot(jnp.broadcast_to(silu_c, (16, D)).astype(BF16), w)[0:1]

    def forward(ut, p_s, o_s, q_s, qrow, kv_s, kvcol):
        def w1_copy(b):
            return pltpu.make_async_copy(w1_hbm.at[:, _span(b, QB)], w1b, sem.at[0])

        gate_c = pltpu.make_async_copy(wmod_hbm.at[:, _span(5, D)], gob, sem.at[10])
        later_c = [wmod_copy(i) for i in range(2, 5)] + [
            pltpu.make_async_copy(wo_hbm, wob, sem.at[12]),
            pltpu.make_async_copy(go_hbm.at[0], go_all, sem.at[20])] + [
            pltpu.make_async_copy(w2_hbm.at[:, _span(b, QB)], w2_all[b], sem.at[16 + b])
            for b in range(NB)]
        _start(later_c, priority=1)

        b1row = b1_ref[...].astype(F32).reshape(1, F)
        ut[:, 0:128] = _col(jnp.concatenate([b1row, jnp.zeros((1, FP - F), F32)], axis=1))[0:F]
        p_s[...] = jnp.zeros(p_s.shape, U32)
        o_s[...] = jnp.ones(o_s.shape, F32)
        wkvt = jnp.concatenate([wkt_ref[...], wvt_ref[...]], axis=0)
        _wait([wmod_copy(0), wmod_copy(1)])
        _start([x_copy(2), x_copy(3), wq_copy()])
        for i in range(2):
            mod_s[i] = modulation(wm_all[_span(i, D), :])
        colv[0] = _col(mod_row(0))
        colv[1] = _col(1.0 + mod_row(1))

        def embed(b, ksq):
            x_copy(b).wait()
            x1t[b] = xb[_span(b, QB), :].T
            hs = []
            for t in range(NT128):
                mu, r, n = _layernorm(x1t[b, :, _lanes(t)].astype(F32))
                stat[b, 0:1, _lanes(t)] = mu
                stat[b, 1:2, _lanes(t)] = r
                hs.append(n * colv[1] + colv[0])
            h = jnp.concatenate(hs, axis=1).astype(BF16)
            ot[pl.ds(b * H, H)] = h.reshape(H, DH, QB)
            kv = _dot(wkvt, h).astype(BF16)
            kt_s[b] = kv[0:DH]
            vt_s[b] = kv[DH:2 * DH]
            kk = kv[0:DH].astype(F32)
            return jnp.maximum(ksq, jnp.sum(kk * kk, axis=0, keepdims=True))

        ksq = jax.lax.fori_loop(0, NB, embed, jnp.zeros((1, QB), F32))
        ksq = jnp.max(ksq, axis=1, keepdims=True)
        wq_copy().wait()
        wqt[...] = wqb[...].T
        build_keys(kt_s, kv_s, kvcol)

        def queries(b):
            q = (_dot(wqt[...], heads(ot, b)) * (SM_SCALE * LOG2E)).astype(BF16)
            qt[pl.ds(b * H, H)] = q.reshape(H, DH, QB)
            q = q.astype(F32).reshape(H, DH, QB)
            shift[_span(b, H), :] = jnp.sum(q * q, axis=1)
            bound = jnp.sqrt(shift[_span(b, H), :] * ksq)
            shift[_span(b, H), :] = bound.astype(BF16).astype(F32)
            return jnp.max(jnp.where(bound <= SAFE_BOUND, 0.0, 1.0)) == 0.0

        def finish(u, acc, l):
            linv = pltpu.reciprocal(_sum0(l), full_range=False)
            rowv[pl.ds(u, 1), :] = linv[0:1]
            ot[u] = (acc * jnp.concatenate([linv, linv], axis=0)).astype(BF16)

        def stage(g):
            first = jax.lax.broadcasted_iota(jnp.int32, (DH, QB), 0) == 0
            for k in range(U):
                qrow[k] = qt[g * U + k].astype(F32)
                aug = jnp.where(first, -shift[pl.ds(g * U + k, 1), :], 0.0)
                q_s[k, 0:DH // 2] = pltpu.bitcast(qt[g * U + k], U32)
                for t in range(NT128):
                    q_s[k, DH // 2:DH, _lanes(t)] = pltpu.bitcast(
                        aug[:, _lanes(t)].astype(BF16), U32)

        def attend_bounded(g, slot):
            neg = [jnp.broadcast_to(-shift[pl.ds(g * U + k, 1), :], (16, QB)) for k in range(U)]
            q_t = [jnp.concatenate([pltpu.bitcast(q_s[k, :, _lanes(t)], BF16)
                                    for t in range(NT128)], axis=1) for k in range(U)]
            always = _true(g)
            ps = {n - LAG: pltpu.bitcast(p_s[n], BF16) for n in range(LAG)}
            acc, l = {-1: o_s[0:DH]}, {-1: o_s[DH:DH + 8]}
            before = jnp.where(g % GB == 0, NU, g * U - 1)

            def values(step, deps):
                k, j = divmod(step, NJ)
                o = _dot(_tie(pltpu.bitcast(keys(vt_s, j), U32), deps, always), ps[step])
                acc[k] = acc[k] + o if j else o
                if j == NJ - 1:
                    finish(g * U + k if k >= 0 else before, acc[k], l[k])

            for step in range(U * NJ):
                k, j = divmod(step, NJ)
                n, deps = BK, []
                if j != LAG and step >= LAG:
                    n = BK - 16
                    tail, deps = _vpu_scores(
                        kvcol.at[j], qrow.at[k], neg[k], (1, 2, 2, 2, 2, 2, 3, 2), 4)
                if step:
                    values(step - LAG, deps)
                s = _dot(key_rows(kv_s, j, 0, n, 2 * DH, deps, always), q_t[k])
                if not step:
                    values(step - LAG, deps)
                head = jnp.exp2(s[0:BK - 16])
                tail = jnp.exp2(tail if n < BK else s[BK - 16:BK])
                ring[slot, step * BK:(step + 1) * BK - 16, :] = head.astype(BF16)
                ring[slot, (step + 1) * BK - 16:(step + 1) * BK, :] = tail.astype(BF16)
                for r in range(0, BK - 16, 8):
                    l[k] = l[k] + head[r:r + 8] if k in l else head[r:r + 8]
                l[k] = l[k] + (tail[0:8] + tail[8:16])
                p = jnp.concatenate([head, tail], axis=0)
                if step + LAG < U * NJ:
                    ps[step] = p.astype(BF16)
                else:
                    for t in range(NT128):
                        p_s[step + LAG - U * NJ, :, _lanes(t)] = pltpu.bitcast(
                            p[:, _lanes(t)].astype(BF16), U32)
            o_s[0:DH] = acc[U - 1]
            o_s[DH:DH + 8] = l[U - 1]
            stage(jnp.where(g % GB == GB - 1, g, g + 1))

        def attend_flush(u):
            acc = o_s[0:DH]
            for n in range(LAG):
                acc = acc + _dot(keys(vt_s, NJ - LAG + n), pltpu.bitcast(p_s[n], BF16))
            finish(u, acc, o_s[DH:DH + 8])

        def attend_exact(g, slot):
            def unit(k, carry):
                u = g * U + k
                m = jax.lax.fori_loop(
                    0, NJ,
                    lambda j, m: jnp.maximum(m, jnp.max(scores(kv_s, u, j), axis=0, keepdims=True)),
                    jnp.full((1, QB), -jnp.inf, F32))
                shift[pl.ds(u, 1), :] = m

                def tile(j, sums):
                    p = jnp.exp2(scores(kv_s, u, j) - m)
                    ring[slot, _span(k * NJ + j, BK), :] = p.astype(BF16)
                    v_t = vt_s[j // NT128, :, _span(j % NT128, BK)]
                    return (sums[0] + _dot(v_t, p.astype(BF16)),
                            sums[1] + jnp.sum(p.reshape(BK // 8, 8, QB), axis=0))

                finish(u, *jax.lax.fori_loop(
                    0, NJ, tile, (jnp.zeros((DH, QB), F32), jnp.zeros((8, QB), F32))))
                return carry

            jax.lax.fori_loop(0, U, unit, 0)

        def group(g, safe):
            i = _kept(g)
            p_move(i >= NSLOT, i - NSLOT, True, lambda cp: cp.wait())
            pl.when(g == NG - 1)(lambda: _start([w1_copy(NB - 1), gate_c]))
            pl.when(safe)(lambda: attend_bounded(g, _slot(i)))
            pl.when(jnp.logical_not(safe))(lambda: attend_exact(g, _slot(i)))
            lo = _spills_before(g)
            p_move(_spills_before(g + 1) > lo, lo, True, lambda cp: cp.start())

        def once():
            _wait(later_c)

            def modulate(i, carry):
                mod_s[i] = modulation(wm_all[_span(i, D), :])
                rows = pl.ds(pl.multiple_of(jnp.minimum((i - 2) * 464, F - 464), 16), 464)
                bias = ut[rows, 0:128]
                for t in range(1, D // 128):
                    ut[rows, _lanes(t)] = bias
                return carry

            jax.lax.fori_loop(2, 5, modulate, 0)
            colv[0] = _col(mod_row(3))
            colv[1] = _col(1.0 + mod_row(4))
            colv[2] = _col(mod_row(2))
            wot[...] = wob[...].T
            b2row = b2_ref[...].astype(F32).reshape(1, S)
            dmod_s[5] = _dot(jnp.broadcast_to(b2row, (16, S)).astype(BF16), go_all[...])[0:1]

            def hidden_cotangent(i, carry):
                for r0, n in ((0, 240), (240, 224)):
                    rows = pl.ds(pl.multiple_of(jnp.minimum(i * 464, F - 464) + r0, 16), n)
                    w2r = jnp.concatenate([w2_all[b][rows, :] for b in range(NB)], axis=1)
                    dut[rows, :] = _dot(w2r, go_all[...]).astype(BF16)
                return carry

            jax.lax.fori_loop(0, 3, hidden_cotangent, 0)

        def block(b, carry):
            pl.when(b < NB - 1)(lambda: w1_copy(b).start())
            safe = queries(b)
            bounded[b] = safe.astype(jnp.int32)
            stage(b * GB)
            jax.lax.fori_loop(b * GB, (b + 1) * GB, lambda g, cc: (group(g, safe), cc)[1], 0)
            pl.when(safe)(lambda: attend_flush((b + 1) * H - 1))
            pl.when(b == 0)(once)
            w1_copy(b).wait()
            a = _dot(wot[...], heads(ot, b))
            ns = []
            for t in range(NT128):
                x1 = (x1t[b, :, _lanes(t)].astype(F32) + colv[2] * a[:, _lanes(t)]).astype(BF16)
                x1t[b, :, _lanes(t)] = x1
                mu2, r2, n2 = _layernorm(x1.astype(F32))
                mu3, r3, n3 = _layernorm(n2 * colv[1] + colv[0])
                stat[b, 2:3, _lanes(t)] = mu2
                stat[b, 3:4, _lanes(t)] = r2
                stat[b, 4:5, _lanes(t)] = mu3
                stat[b, 5:6, _lanes(t)] = r3
                ns.append(n3)
            early, late = jnp.concatenate(ns[0:2], axis=1), jnp.concatenate(ns[2:4], axis=1)
            left, right = slice(0, D // 2), slice(D // 2, D)
            b11, b12, b21, b22 = early[left], early[right], late[left], late[right]
            chunks = [(slice(sum(ROWS[:c]), sum(ROWS[:c + 1])),
                       slice(F // 2 + sum(ROWS[:c]), F // 2 + sum(ROWS[:c + 1])))
                      for c in range(len(ROWS))]
            r2, r6 = b11.astype(BF16), (b11 + b12).astype(BF16)
            for top, low in chunks:
                p2 = _dot(_plus(w1b[low, left], w1b[low, right]), r2, NT)
                p6 = _dot(_plus(w1b[low, left], w1b[top, left], -1), r6, NT)
                ut[low, left] += p2
                ut[low, right] += p6 - p2
            r1, r3, r4, r5, r7 = (
                v.astype(BF16) for v in (b11 + b22, b12 - b22, b21 - b11, b22, b21 + b22))
            for top, low in chunks:
                a11, a12, a22 = w1b[top, left], w1b[top, right], w1b[low, right]
                p1 = _dot(_plus(a11, a22), r1, NT)
                p3 = _dot(a11, r3, NT)
                ut[low, right] += p1 + p3
                p4 = _dot(a22, r4, NT)
                ut[low, left] += p4
                p5 = _dot(_plus(a11, a12), r5, NT)
                ut[top, right] += p3 + p5
                ut[top, left] += p1 + p4 - p5 + _dot(_plus(a12, a22, -1), r7, NT)
            return carry

        jax.lax.fori_loop(0, NB, block, 0)

        gate_c.wait()
        mod_s[5] = modulation(gob[...])
        go_copy(NB - 1).start()
        gate = jnp.broadcast_to(mod_row(5), (16, D))

        def gelu(r0, dgate):
            rows = pl.ds(r0, 16)
            u = ut[rows, :]
            u2 = u * u
            half = 0.5 * jnp.tanh(u * (GELU_C + (GELU_C * GELU_A) * u2)) + 0.5
            g = u * half
            dgelu = half + (g * (1.0 - half)) * (2.0 * GELU_C + (6.0 * GELU_C * GELU_A) * u2)
            e = dut[rows, :].astype(F32)
            gt[rows, :] = (g * gate).astype(BF16)
            dut[rows, :] = (e * gate * dgelu).astype(BF16)
            return dgate + g * e

        stride = F // 4 // 16 * 16

        def gelu_rows(i, dgate):
            for r in range(0, stride, 16):
                dgate = gelu(pl.multiple_of(i * stride + r, 16), dgate)
            return dgate

        dgate = jax.lax.fori_loop(0, 4, gelu_rows, jnp.zeros((16, D), F32))
        for r in range(4 * stride, F, 16):
            dgate = gelu(r, dgate)
        dmod_s[5] += jnp.sum(dgate, axis=0, keepdims=True)

    pl.run_scoped(forward, pltpu.VMEM((F, D), F32),
                  pltpu.VMEM((LAG, BK // 2, QB), U32), pltpu.VMEM((DH + 8, QB), F32),
                  pltpu.VMEM((U, DH, QB), U32), pltpu.VMEM((U, DH, QB), F32), *key_buffers())

    wo_again = pltpu.make_async_copy(wo_hbm, gob, sem.at[13])

    def dense_backward(dw1b, w2b, dn3_s, got, n3b, wog, b2_s, db2_s, sums_s, head_s):
        def w_copies(src, dst, first_sem, b, half):
            edges = (0, 352, F // 2, 1040, F)
            return [pltpu.make_async_copy(src.at[edges[n]:edges[n + 1], _span(b, QB)],
                                          dst.at[edges[n]:edges[n + 1], :], sem.at[first_sem + n])
                    for n in (2 * half, 2 * half + 1)]

        def w1_copies(b):
            return w_copies(w1_hbm, w1b, 5, b, 0) + w_copies(w1_hbm, w1b, 5, b, 1)

        def w2_copies(b, half):
            return w_copies(w2_hbm, w2b, 9, b, half)

        def out_copy(b):
            return pltpu.make_async_copy(gob, out_hbm.at[0, _span(b, QB), :], sem.at[14])

        def dw1_copy(b):
            return pltpu.make_async_copy(dw1b, dw1_hbm.at[:, _span(b, QB)], sem.at[1])

        def dw2_copy(b, half):
            return pltpu.make_async_copy(
                w2b.at[half * F:half * F + F // 2, :],
                dw2_hbm.at[_span(half, F // 2), _span(b, QB)], sem.at[3 + half])

        def hidden(ref, n, half):
            rest = jnp.concatenate([ref[256:F, _span(half, D // 2)],
                                    jnp.zeros((FP - F, D // 2), BF16)], axis=0).T
            return jnp.concatenate([head_s[n, half], pltpu.bitcast(rest, U32)], axis=1)

        wo_c = pltpu.make_async_copy(wo_hbm, wog, sem.at[15])
        _start([wo_c] + w2_copies(NB - 1, 0) + w2_copies(NB - 1, 1))
        for n, ref in enumerate((dut, gt)):
            head = pltpu.bitcast(ref[0:256, :].T, U32)
            head_s[n, 0] = head[0:D // 4]
            head_s[n, 1] = head[D // 4:D // 2]
        b1_ref[...] = _dot(jnp.ones((16, D), BF16), dut[...], NT)[0:1].reshape(F).astype(BF16)
        colv[2] = _col(mod_row(5))
        b2row = b2_ref[...].astype(F32).reshape(1, S)
        for b in range(NB):
            b2_s[b] = b2row[:, b * QB:(b + 1) * QB]
        acc_s[...] = jnp.zeros(acc_s.shape, F32)

        def block(bi, carry):
            b = NB - 1 - bi
            pl.when(bi > 0)(lambda: _wait(w1_copies(b)))
            go_copy(b).wait()

            def stats(cols):
                rows = [stat[b, k:k + 1, cols] for k in range(2, 6)]
                return [jnp.broadcast_to(r, (8, r.shape[1])) for r in rows]

            s1 = s2 = jnp.zeros((8, QB), F32)
            for half in range(2):
                dn3 = _dot(pltpu.bitcast(hidden(dut, 0, half), BF16)[:, 0:F], w1b[...])
                got[_span(half, D // 2), :] = gob[:, _span(half, D // 2)].T
                dn3_s[_span(half, D // 2), :] = dn3
                mu2, r2, mu3, r3 = stats(slice(None))
                for r in range(0, D // 2, 8):
                    rows = pl.ds(half * (D // 2) + r, 8)
                    n2 = (x1t[b, rows, :].astype(F32) - mu2) * r2
                    n3 = (n2 * _wide(colv[1, rows]) + _wide(colv[0, rows]) - mu3) * r3
                    n3b[rows, :] = n3.astype(BF16)
                    s1 = s1 + dn3[r:r + 8]
                    s2 = s2 + dn3[r:r + 8] * n3
            sums_s[0] = _sum0(s1) * (1.0 / D)
            sums_s[1] = _sum0(s2) * (1.0 / D)
            _wait(w2_copies(b, 0) + w2_copies(b, 1))
            pl.when(bi > 0)(lambda: _wait([dw2_copy(b + 1, 1), dw1_copy(b + 1)]))
            pl.when(b > 0)(lambda: _start(w1_copies(b - 1)))

            for half in range(2):
                always = _true(b)
                deps, later = [], []
                for t in range(half * NT128 // 2, (half + 1) * NT128 // 2):
                    cols = _lanes(t)
                    mu2, r2, mu3, r3 = stats(cols)
                    m1, m2 = sums_s[0, :, cols], sums_s[1, :, cols]
                    dn2s = []
                    for r in range(0, D, 8):
                        n2 = (x1t[b, r:r + 8, cols].astype(F32) - mu2) * r2
                        scale = colv[1, r:r + 8]
                        n3 = (n2 * scale + colv[0, r:r + 8] - mu3) * r3
                        dh2 = r3 * (dn3_s[r:r + 8, cols] - m1 - n3 * m2)
                        dhn = dh2 * n2
                        acc_s[0, r:r + 8] += dh2
                        acc_s[1, r:r + 8] += dhn
                        dn2s.append(dh2 * scale)
                        t1 = t1 + dn2s[-1] if r else dn2s[-1]
                        t2 = t2 + dhn * scale if r else dhn * scale
                        deps.append(t2)
                    later.append(
                        (cols, mu2, r2, _sum0(t1) * (1.0 / D), _sum0(t2) * (1.0 / D), dn2s))
                rows = _span(half, D // 2)
                g = pltpu.bitcast(_after(hidden(gt, 1, half), deps, always), BF16)
                y = _dot(g[:, 0:F], w2b[0:F, :])
                bias = b2_s[b]
                gob[:, rows] = jnp.concatenate(
                    [x1t[b, rows, _lanes(t)].astype(F32) + colv[2, rows] * bias[:, _lanes(t)]
                     + y[:, _lanes(t)] for t in range(NT128)], axis=1).astype(BF16).T
                deps = []
                for cols, mu2, r2, t1, t2, dn2s in later:
                    for r in range(0, D, 8):
                        n2 = (x1t[b, r:r + 8, cols].astype(F32) - mu2) * r2
                        go = got[r:r + 8, cols].astype(F32)
                        db2 = db2 + go * colv[2, r:r + 8] if r else go * colv[2, 0:8]
                        deps.append(go + r2 * (dn2s[r // 8] - t1 - n2 * t2))
                        dn3_s[r:r + 8, cols] = deps[-1]
                    db2_s[b, :, cols] = jnp.sum(db2, axis=0, keepdims=True)
                du = _after(pltpu.bitcast(dut[_span(half, F // 2), :], U32), deps, always)
                dw1b[_span(half, F // 2), :] = _dot(pltpu.bitcast(du, BF16), n3b[...]).astype(BF16)

            @pl.when(bi == 0)
            def _():
                wo_c.wait()
                wog[...] = (wog[...].astype(F32) * mod_row(2)).astype(BF16)

            _start([out_copy(b), dw1_copy(b)])
            pl.when(b > 0)(lambda: _start(w2_copies(b - 1, 1)))
            rhs = _strassen_rhs(got[...])
            for c, n in enumerate(ROWS):
                r = sum(ROWS[:c])
                parts = _strassen(gt[r:r + n, :], gt[F // 2 + r:F // 2 + r + n, :], rhs)
                for half, part in enumerate(parts):
                    w2b[half * F + r:half * F + r + n, :] = part.astype(BF16)
            out_copy(b).wait()
            pl.when(b > 0)(lambda: go_copy(b - 1).start())
            pl.when(b == 0)(lambda: wo_again.start())
            _start([dw2_copy(b, 0), dw2_copy(b, 1)])

            o_b = heads(ot, b)
            dx1 = dn3_s[...].astype(BF16)
            do = _dot(wog[...], dx1)
            gacc[...] = jnp.where(bi > 0, gacc[...], 0.0) + _dot(o_b, dx1, NT)
            for r in range(0, D, 8):
                x1t[b, r:r + 8, :] = dn3_s[r:r + 8, :].astype(BF16)
            linv = rowv[_span(b, H), :]
            dos, deltas = [], []
            for h in range(H):
                doh = (do[h * DH:(h + 1) * DH] * linv[h:h + 1]).astype(BF16)
                deltas.append(jnp.sum(doh.astype(F32) * o_b[h * DH:(h + 1) * DH].astype(F32),
                                      axis=0, keepdims=True))
                dos.append(doh)
            rowv[_span(b, H), :] = jnp.concatenate(deltas, axis=0)
            ot[pl.ds(b * H, H)] = jnp.stack(dos)
            dw2_copy(b, 0).wait()
            pl.when(b > 0)(lambda: _start(w2_copies(b - 1, 0)))
            return carry

        jax.lax.fori_loop(0, NB, block, 0)
        b2_ref[...] = jnp.concatenate(
            [db2_s[b] for b in range(NB)], axis=1).reshape(S).astype(BF16)
        _wait([dw2_copy(0, 1), dw1_copy(0)])

    pl.run_scoped(dense_backward,
                  pltpu.VMEM((F, QB), BF16), pltpu.VMEM((F + F // 2, QB), BF16),
                  pltpu.VMEM((D, QB), F32), pltpu.VMEM((D, QB), BF16), pltpu.VMEM((D, QB), BF16),
                  pltpu.VMEM((D, D), BF16), pltpu.VMEM((NB, 1, QB), F32),
                  pltpu.VMEM((NB, 1, QB), F32), pltpu.VMEM((2, 8, QB), F32),
                  pltpu.VMEM((2, 2, D // 4, 256), U32))

    dwo_c = pltpu.make_async_copy(dwob, dwo_hbm, sem.at[22])

    def attention_backward(dkv, ds_s, dst_s, dq_s, do_s, qrow, v_s, vcol, k_s, kcol):
        wo_again.wait()
        build_keys(vt_s, v_s, vcol)
        colv[0] = _col(mod_row(0))
        colv[1] = _col(1.0 + mod_row(1))
        colv[2] = _col(silu_c)
        for i in range(2):
            dmod_s[3 + i] = _row(acc_s[i])
        dwob[...] = (gacc[...] * mod_row(2)).astype(BF16)
        dmod_s[2] = jnp.sum(gob[...].astype(F32) * gacc[...], axis=0, keepdims=True)
        dkv[...] = jnp.zeros(dkv.shape, F32)
        ds_s[...] = jnp.zeros(ds_s.shape, U32)
        dst_s[...] = jnp.zeros(dst_s.shape, U32)
        dq_s[...] = jnp.zeros(dq_s.shape, F32)
        qt[NU] = jnp.zeros((DH, QB), BF16)
        dwo_c.start()

        def recompute_bounded(r, carry):
            u0 = (REC0 + r) * U
            for k in range(U):
                qrow[k] = qt[u0 + k].astype(F32)
            always = _true(r)
            for k in range(U):
                m = shift[pl.ds(u0 + k, 1), :]
                neg = jnp.broadcast_to(-m, (16, QB))
                for j in range(NJ):
                    tail, deps = _vpu_scores(kcol.at[j], qrow.at[k], neg, (1,) * 7, 4)
                    s = _dot(key_rows(k_s, j, 0, BK - 16, DH, deps, always), qt[u0 + k])
                    r0 = k * S + j * BK
                    ring[GB + 2 + r, r0:r0 + BK - 16, :] = jnp.exp2(s - m).astype(BF16)
                    ring[GB + 2 + r, r0 + BK - 16:r0 + BK, :] = jnp.exp2(tail).astype(BF16)
            return carry

        def recompute_exact(n, carry):
            u = REC0 * U + n // NJ
            ring[GB + 2 + n // (U * NJ), _span(n % (U * NJ), BK), :] = jnp.exp2(
                scores(k_s, u, n % NJ) - shift[pl.ds(u, 1), :]).astype(BF16)
            return carry

        def flip(ds):
            return pltpu.bitcast(ds.T, U32)

        def late_scores(n):
            ds = pltpu.bitcast(ds_s[n], BF16)
            return ds, dst_s[n] if n < LAG - 1 else flip(ds)

        def query_key_grads(j, ds, q_t, deps, always):
            dq = _dot(_tie(pltpu.bitcast(keys(kt_s, j), U32), deps, always), ds[0])
            dkv[0:DH, j * BK:(j + 1) * BK] += _dot(
                _tie(pltpu.bitcast(q_t, U32), deps, always), pltpu.bitcast(ds[1], BF16))
            return dq

        def stage(g):
            for k in range(UB):
                do_s[k] = ot[g * U + k].astype(F32)

        def groups(n, carry):
            g = NG - PAIR * (n + 1)
            kept = [_kept(g + a) for a in range(PAIR)]
            redo = [jnp.logical_and(g + a >= REC0, g + a < GB) for a in range(PAIR)]

            @pl.when(g == GB - PAIR)
            def _():
                build_keys(kt_s, k_s, kcol)
                _start([x_copy(b) for b in range(NB)] + [wq_copy()])
                jax.lax.fori_loop(0, bounded[0] * NREC, recompute_bounded, 0)
                jax.lax.fori_loop(0, (1 - bounded[0]) * NREC * U * NJ, recompute_exact, 0)
                _start([wmod_copy(i) for i in range(6)])

            for i, r in zip(kept, redo):
                p_move(jnp.logical_and(i < NSPILL, jnp.logical_not(r)), i, False,
                       lambda cp: cp.wait())
            slots = [jnp.where(redo[a], GB + 2 + g + a - REC0, _slot(kept[a])) for a in range(PAIR)]

            def probs(step):
                a, r0 = divmod(step * BK, U * S)
                return ring[slots[a], r0:r0 + BK, :]

            q_t = [qt[g * U + k] for k in range(UB)]
            do_t = [ot[g * U + k] for k in range(UB)]
            delta = [rowv[pl.ds(g * U + k, 1), :] for k in range(UB)]
            neg = [jnp.broadcast_to(-d, (16, QB)) for d in delta]
            before = jnp.where(n == 0, NU, g * U + 2 * UB - 1)
            always = _true(g)
            ds = {m - LAG: late_scores(m) for m in range(LAG)}
            dq = {-1: dq_s[...]}
            q_t.append(qt[before])
            for step in range(UB * NJ):
                k, j = divmod(step, NJ)
                kl, jl = divmod(step - LAG, NJ)
                last, deps = BK, []
                if step >= LAG:
                    last = BK - 16
                    tail, deps = _vpu_scores(
                        vcol.at[j], do_s.at[k], neg[k], (3, 4, 4, 3, 3, 3, 3, 4, 5, 5), 2)
                split = 64 if step < UB * NJ - 1 else last
                p = probs(step)
                dp = [_dot(key_rows(v_s, j, 0, split, DH, deps, always), do_t[k]) - delta[k]]
                dkv[DH:2 * DH, j * BK:(j + 1) * BK] += _dot(
                    _tie(pltpu.bitcast(do_t[k], U32), deps, always), p, NT)
                if split < last:
                    dp.append(
                        _dot(key_rows(v_s, j, split, last, DH, deps, always), do_t[k]) - delta[k])
                if last < BK:
                    dp.append(tail)
                full = probs(step).astype(F32) * jnp.concatenate(dp, axis=0)
                m = step + LAG - UB * NJ
                if m < 0:
                    full = full.astype(BF16)
                    ds[step] = full, flip(full)
                else:
                    words = jnp.concatenate([pltpu.bitcast(full[:, _lanes(t)].astype(BF16), U32)
                                             for t in range(NT128)], axis=1)
                    ds_s[m] = words
                    if m < LAG - 1:
                        dst_s[m] = flip(pltpu.bitcast(words, BF16))
                r = query_key_grads(jl, ds[step - LAG], q_t[kl], deps, always)
                dq[kl] = dq[kl] + r if jl else r
                if jl == NJ - 1:
                    qt[g * U + kl if kl >= 0 else before] = (dq[kl] * SM_SCALE).astype(BF16)
            dq_s[...] = dq[UB - 1]
            stage(jnp.maximum(g - PAIR, 0))
            for i in kept[::-1]:
                p_move(i >= NSLOT, i - NSLOT, False, lambda cp: cp.start(priority=1))
            return carry

        stage(NG - PAIR)
        jax.lax.fori_loop(0, NG // PAIR, groups, 0)
        dq = dq_s[...]
        for n in range(LAG):
            dq = dq + query_key_grads(NJ - LAG + n, late_scores(n), qt[UB - 1], [], None)
        qt[UB - 1] = (dq * SM_SCALE).astype(BF16)
        for b in range(NB):
            kt_s[b] = (dkv[0:DH, b * QB:(b + 1) * QB] * (1.0 / LOG2E)).astype(BF16)
            vt_s[b] = dkv[DH:2 * DH, b * QB:(b + 1) * QB].astype(BF16)

    pl.run_scoped(attention_backward,
                  pltpu.VMEM((2 * DH, S), F32), pltpu.VMEM((LAG, BK // 2, QB), U32),
                  pltpu.VMEM((LAG - 1, QB // 2, BK), U32), pltpu.VMEM((DH, QB), F32),
                  pltpu.VMEM((UB, DH, QB), F32), pltpu.VMEM((U, DH, QB), F32),
                  *key_buffers(), *key_buffers())

    def input_backward(dn1_s, t_s, xt_s):
        wkv = jnp.concatenate(
            [wkt_ref[...].astype(F32), wvt_ref[...].astype(F32),
             jnp.zeros((128 - 2 * DH, D), F32)], axis=0).T[:, 0:2 * DH].astype(BF16)
        _wait([x_copy(b) for b in range(NB)] + [wq_copy()] + [wmod_copy(i) for i in range(6)])

        def dwmod_copy(i):
            return pltpu.make_async_copy(
                dwm_all.at[_span(i, D), :], dwmod_hbm.at[:, _span(i, D)], sem.at[16 + i])

        def dx_copy(b):
            return pltpu.make_async_copy(
                xb.at[_span(b, QB), :], dx_hbm.at[0, _span(b, QB), :], sem.at[1 + b])

        def dwmod(i):
            row = dmod_s[i]
            dwm_all[_span(i, D), :] = jnp.concatenate(
                [colv[2] * row[:, _lanes(t)] for t in range(D // 128)], axis=1).astype(BF16)
            dwmod_copy(i).start()

        def cond_grad(i, t):
            row = jnp.broadcast_to(dmod_s[i][:, _lanes(t)], (16, 128)).astype(BF16)
            return _dot(row, wm_all[_span(i, D), _lanes(t)], NT)

        def stats(b):
            return [jnp.broadcast_to(stat[b, k:k + 1, :], (8, QB)) for k in range(2)]

        def hidden_grad(b, dsilu):
            xt = xb[_span(b, QB), :].T
            xt_s[b] = pltpu.bitcast(xt, U32)
            mu1, r1 = stats(b)
            n1s, hs, deps = {}, {}, []
            for t in range(NT128):
                for u in range(H):
                    rows = slice(u * DH, (u + 1) * DH)
                    n1s[u, t] = (xt[rows, _lanes(t)].astype(F32)
                                 - mu1[0:1, _lanes(t)]) * r1[0:1, _lanes(t)]
                    hs[u, t] = n1s[u, t] * colv[1, rows] + colv[0, rows]
                    if t % 2:
                        ot[b * H + u, :, (t - 1) * 128:(t + 1) * 128] = jnp.concatenate(
                            [hs[u, t - 1], hs[u, t]], axis=1).astype(BF16)
                    deps.append(hs[u, t][8:16])
            w = pltpu.bitcast(_after(pltpu.bitcast(wqb[...], U32),
                                     deps + deps[-1:] * (len(deps) // 3), _true(b)), BF16)
            dq = heads(qt, b)
            dh = _dot(wkv, jnp.concatenate([kt_s[b], vt_s[b]], axis=0))
            for t in range(D // 128):
                dsilu = dsilu + cond_grad(2 + b, t)
                dh = dh + _dot(w[:, _lanes(t)], dq[_lanes(t), :])
            for r in range(0, D, 8):
                rows = slice(r, r + 8)
                scale = _wide(colv[1, rows])
                dhn = dh[rows] * jnp.concatenate(
                    [n1s[r // DH, t][r % DH:r % DH + 8] for t in range(NT128)], axis=1)
                acc_s[0, rows] = sum((dh[rows, _lanes(t)] for t in range(NT128)),
                                     jnp.where(b > 0, acc_s[0, rows], 0.0))
                acc_s[1, rows] = sum((dhn[:, _lanes(t)] for t in range(NT128)),
                                     jnp.where(b > 0, acc_s[1, rows], 0.0))
                dn1 = dh[rows] * scale
                dn1_s[b, rows, :] = dn1
                t1 = t1 + dn1 if r else dn1
                t2 = t2 + dhn * scale if r else dhn * scale
            t_s[b, 0] = _sum0(t1) * (1.0 / D)
            t_s[b, 1] = _sum0(t2) * (1.0 / D)
            dwmod(2 + b)
            return dsilu

        def input_grad(b, carry):
            mu1, r1 = stats(b)
            c2 = t_s[b, 1] * r1
            c1 = t_s[b, 0] - mu1 * c2
            deps = []
            for t in range(NT128):
                cols, dxs = _lanes(t), []
                for r in range(0, D, 16):
                    x = pltpu.bitcast(xt_s[b, r // 2:r // 2 + 8, cols], BF16).astype(F32)
                    dxs.append(x1t[b, r:r + 16, cols].astype(F32) + r1[0:1, cols] * (
                        dn1_s[b, r:r + 16, cols] - c1[0:1, cols] - x * c2[0:1, cols]))
                    deps.append(dxs[-1][8:16])
                xb[_span(b * NT128 + t, 128), :] = jnp.concatenate(dxs, axis=0).astype(BF16).T
            h = _after(pltpu.bitcast(heads(ot, b), U32),
                       deps + deps[-1:] * (len(deps) // 4), _true(b))
            gacc[...] = jnp.where(b > 0, gacc[...], 0.0) + _dot(
                pltpu.bitcast(h, BF16), heads(qt, b), NT)
            dx_copy(b).start()
            return carry

        dsilu = jax.lax.fori_loop(0, NB, hidden_grad, jnp.zeros((16, D), F32))
        for i in range(2):
            dmod_s[i] = _row(acc_s[i])
            dwmod(i)
        jax.lax.fori_loop(0, NB, input_grad, 0)
        dwqb[...] = gacc[...].astype(BF16)
        dwq_c = pltpu.make_async_copy(dwqb, dwq_hbm, sem.at[11])
        dwq_c.start()
        dwkv = sum(_dot(jnp.concatenate([kt_s[b], vt_s[b]], axis=0), heads(ot, b), NT)
                   for b in range(NB))
        dsilu = sum((cond_grad(i, t) for i in range(2) for t in range(D // 128)), dsilu)
        c_ref[...] = (dsilu[0:1] * (sig * (1.0 + c32 * (1.0 - sig)))).astype(BF16)
        wkt_ref[...] = dwkv[0:DH].astype(BF16)
        wvt_ref[...] = dwkv[DH:2 * DH].astype(BF16)
        _start(small_out)
        _wait([dwo_c] + [dwmod_copy(i) for i in range(6)] + [dx_copy(b) for b in range(NB)]
              + [dwq_c] + small_out)

    pl.run_scoped(input_backward, pltpu.VMEM((NB, D, QB), F32), pltpu.VMEM((NB, 2, 8, QB), F32),
                  pltpu.VMEM((NB, D // 2, QB), U32))


@jax.jit
def pallas_adaLN_cond__grouped_kv_mqa__mixer_token_mlp__prompt_kernel(
    A_x: jax.Array,
    A_wq: jax.Array,
    A_wk: jax.Array,
    A_wv: jax.Array,
    A_wo: jax.Array,
    B_x: jax.Array,
    B_w1: jax.Array,
    B_b1: jax.Array,
    B_w2: jax.Array,
    B_b2: jax.Array,
    c: jax.Array,
    w_mod: jax.Array,
    grad_out: jax.Array,
):
    del B_x
    hbm = pl.BlockSpec(memory_space=pl.ANY)

    def sds(*shape):
        return jax.ShapeDtypeStruct(shape, BF16)

    (out, dx, dwq, dwkt, dwvt, dwo, dw1t, db1, dw2, db2, dc, dwmod, _) = pl.pallas_call(
        _kernel,
        in_specs=[hbm] * 12,
        out_specs=[hbm] * 13,
        out_shape=[sds(1, S, D), sds(1, S, D), sds(D, D), sds(DH, D), sds(DH, D), sds(D, D),
                   sds(F, S), sds(F), sds(F, S), sds(S), sds(1, D), sds(D, 6 * D),
                   sds(NSPILL * U * S - EXTRA, QB)],
        scratch_shapes=[
            pltpu.VMEM((NSLOT, U * S, QB), BF16),
            pltpu.VMEM((EXTRA, QB), BF16),
            pltpu.VMEM((NB, D, QB), BF16),
            pltpu.VMEM((NU + 1, DH, QB), BF16),
            pltpu.VMEM((NU + 1, DH, QB), BF16),
            pltpu.VMEM((NB, DH, QB), BF16),
            pltpu.VMEM((NB, DH, QB), BF16),
            pltpu.VMEM((NU + 8, QB), F32),
            pltpu.VMEM((NU, QB), F32),
            pltpu.VMEM((NB, 8, QB), F32),
            pltpu.VMEM((6, 1, D), F32),
            pltpu.VMEM((6, 1, D), F32),
            pltpu.VMEM((3, D, 128), F32),
            pltpu.VMEM((F, QB), BF16),
            pltpu.VMEM((F, D), BF16),
            pltpu.VMEM((F, D), BF16),
            pltpu.VMEM((QB, D), BF16),
            pltpu.VMEM((D, D), F32),
            pltpu.VMEM((2, D, 128), F32),
            pltpu.VMEM((DH, D), BF16), pltpu.VMEM((DH, D), BF16), pltpu.VMEM((F,), BF16),
            pltpu.VMEM((S,), BF16), pltpu.VMEM((1, D), BF16),
            pltpu.SMEM((NB,), jnp.int32),
            pltpu.SemaphoreType.DMA((NSLOT + 1,)),
            pltpu.SemaphoreType.DMA((28,)),
        ],
        compiler_params=pltpu.CompilerParams(
            vmem_limit_bytes=128 * 1024 * 1024, disable_bounds_checks=True),
        name="adaln_mqa_mixer_fwd_bwd",
    )(A_x, A_wq, A_wk.T, A_wv.T, A_wo, B_w1.T, B_b1, B_w2, B_b2, c, w_mod, grad_out)
    return (out, dx, dwq, dwkt.T, dwvt.T, dwo, dw1t.T, db1, dw2, db2, dc, dwmod)
```
